```python
import jax
import jax.numpy as jnp

def _softmax(x, axis=-1):
    return jax.nn.softmax(x, axis=axis)

def _gelu(x):
    return jax.nn.gelu(x, approximate=True)

def _silu(x):
    return jax.nn.silu(x)

def _sigmoid(x):
    return jax.nn.sigmoid(x)

def _layernorm(x, axis=-1, eps=1e-05):
    m = jnp.mean(x, axis=axis, keepdims=True)
    v = jnp.var(x, axis=axis, keepdims=True)
    return (x - m) / jnp.sqrt(v + eps)

def _scatter_add(tgt, idx, src, axis=0):
    return tgt.at[idx].add(src)

def _segment_sum(src, seg, n):
    return jax.ops.segment_sum(src, seg, n)

class _Rng:

    def __init__(self, key):
        self._k = key

    def _next(self):
        self._k, sub = jax.random.split(self._k)
        return sub

    def normal(self, shape):
        return jax.random.normal(self._next(), shape, dtype=jnp.bfloat16)

    def randint(self, lo, hi, shape):
        return jax.random.randint(self._next(), shape, lo, hi, dtype=jnp.int32)

    def uniform(self, shape, lo=0.0, hi=1.0):
        return jax.random.uniform(self._next(), shape, jnp.bfloat16, lo, hi)

    def permutation(self, n):
        return jax.random.permutation(self._next(), n)
kernel_name = 'standalone__dilated_atrous__vision'

def setup_inputs():
    _rng = _Rng(jax.random.key(int.from_bytes(__import__("os").urandom(4), "little")))
    _w = lambda a: (lambda t: t.astype(jnp.bfloat16) if jnp.issubdtype(t.dtype, jnp.floating) else t)(jnp.asarray(a))
    H = W = 384
    C = 384
    k = 1
    return {'x': _w((lambda *s: _rng.normal(s) * 0.05)(1, H, W, C)), 'w': _w((lambda *s: _rng.normal(s) * 0.05)(k, k, C, C) * (1.0 / (k * C ** 0.5)))}

def reference(x, w):
    B, H, W, C = x.shape
    k = 1
    rate = 2
    pad = (k - 1) * rate // 2
    xp = jnp.pad(x, ((0, 0), (pad, pad), (pad, pad), (0, 0)))
    out = jnp.zeros_like(x)
    for i in range(k):
        for j in range(k):
            tap = xp[:, i * rate:i * rate + H, j * rate:j * rate + W, :].copy()
            out = out + jnp.einsum('bhwc,co->bhwo', tap, w[i, j])
    return out
```

```python
import jax
import jax.numpy as jnp
from jax import lax
import jax.experimental.pallas as pl
import jax.experimental.pallas.tpu as pltpu

_S = 32
_B = 64
_PU = 36
_F = 2


@jax.jit
def pallas_standalone__dilated_atrous__vision_kernel(x: jax.Array, w: jax.Array):
    B, H, W, C = x.shape
    O = w.shape[-1]
    M = B * H * W
    S, b, Pu, F = _S, _B, _PU, _F
    n = M // (S * b)
    assert n * S * b == M and n % Pu == 0
    G = n // Pu
    A = F + 1
    T = F + 1
    NX = NO = Pu // 2 + A + 2
    hs = S // 2
    nE = 2 * n

    def kernel(x_hbm, w_hbm, o_hbm, xbuf, obuf, wbuf, rsem, osem, wsem):
        def rd(c):
            s = lax.rem(c, NX)
            rows = pl.ds(pl.multiple_of(c * b, b), b)
            return pltpu.make_async_copy(x_hbm.at[:, rows], xbuf.at[s], rsem.at[s])

        def wr(c):
            s = lax.rem(c, NO)
            rows = pl.ds(pl.multiple_of(c * b, b), b)
            return pltpu.make_async_copy(obuf.at[s], o_hbm.at[:, rows], osem.at[s])

        def decode(i):
            ip = jnp.maximum(i - A, 0)
            k = lax.div(ip, 2 * Pu)
            r = ip - k * (2 * Pu)
            nr = jnp.where(k == G - 1, Pu - A, Pu)
            is_rd = jnp.logical_or(i < A, r < nr)
            c = jnp.where(i < A, i, jnp.where(r < nr, A + k * Pu + r, k * Pu + r - nr))
            return is_rd, c

        def apply(i, fn):
            is_rd, c = decode(i)
            pl.when(is_rd)(lambda: fn(rd(c)))
            pl.when(jnp.logical_not(is_rd))(lambda: fn(wr(c)))

        wcopy = pltpu.make_async_copy(w_hbm, wbuf, wsem.at[0])
        wcopy.start()
        for i in range(F):
            rd(jnp.int32(i)).start()
        wcopy.wait()

        def step(j, _):
            pl.when(j < nE - T)(lambda: apply(j, lambda d: d.wait()))
            pl.when(j + F < nE - T)(lambda: apply(j + F, lambda d: d.start()))
            u = lax.div(j, 2)
            h = j - 2 * u
            xv = xbuf[lax.rem(u, NX), pl.ds(h * hs, hs)].reshape(hs * b, C)
            r = jnp.dot(xv, wbuf[...], preferred_element_type=jnp.float32)
            obuf[lax.rem(u, NO), pl.ds(h * hs, hs)] = r.astype(obuf.dtype).reshape(hs, b, O)
            pl.when(jnp.logical_and(h == 1, u >= n - T))(lambda: wr(u).start())

        lax.fori_loop(0, nE, step, None)
        for c in range(n - T, n):
            wr(jnp.int32(c)).wait()

    out = pl.pallas_call(
        kernel,
        in_specs=[pl.BlockSpec(memory_space=pl.ANY), pl.BlockSpec(memory_space=pl.ANY)],
        out_specs=pl.BlockSpec(memory_space=pl.ANY),
        out_shape=jax.ShapeDtypeStruct((S, M // S, O), x.dtype),
        scratch_shapes=[
            pltpu.VMEM((NX, S, b, C), x.dtype),
            pltpu.VMEM((NO, S, b, O), x.dtype),
            pltpu.VMEM((C, O), w.dtype),
            pltpu.SemaphoreType.DMA((NX,)),
            pltpu.SemaphoreType.DMA((NO,)),
            pltpu.SemaphoreType.DMA((1,)),
        ],
        compiler_params=pltpu.CompilerParams(vmem_limit_bytes=100 * 1024 * 1024),
    )(x.reshape(S, M // S, C), w.reshape(C, O))
    return out.reshape(B, H, W, O)
```

```python
import jax
import jax.numpy as jnp
from jax import lax
import jax.experimental.pallas as pl
import jax.experimental.pallas.tpu as pltpu

_S = 8
_BU = 128
_P = 72
_D = 3
_E = 1
_RD = (4, 32)
_WR = (8, 32)


def _loop(lo, hi, fn):
    def body(j, carry):
        fn(j)
        return carry

    lax.fori_loop(lo, hi, body, None)


@jax.jit
def pallas_standalone__dilated_atrous__vision_kernel(x: jax.Array, w: jax.Array):
    B, H, W, C = x.shape
    O = w.shape[-1]
    M = B * H * W
    S, bu, P, D, E = _S, _BU, _P, _D, _E
    n = M // (S * bu)
    assert n * S * bu == M and n % P == 0 and P % 2 == 0
    G = n // P
    half = P // 2

    def kernel(x_hbm, w_hbm, o_hbm, xbuf, obuf, wbuf, rsem, osem, wsem):
        def pieces(shape):
            ns, nr = shape
            return [(s0, ns, r0, nr) for r0 in range(0, bu, nr) for s0 in range(0, S, ns)]

        def read_start(k, j):
            off = (k * P + j) * bu
            for i, (s0, ns, r0, nr) in enumerate(pieces(_RD)):
                pltpu.make_async_copy(
                    x_hbm.at[pl.ds(s0, ns), pl.ds(pl.multiple_of(off + r0, nr), nr)],
                    xbuf.at[j, pl.ds(s0, ns), pl.ds(r0, nr)],
                    rsem.at[j],
                ).start(priority=i % 2)

        def write_start(k, j):
            off = (k * P + j) * bu
            for s0, ns, r0, nr in pieces(_WR):
                pltpu.make_async_copy(
                    obuf.at[j, pl.ds(s0, ns), pl.ds(r0, nr)],
                    o_hbm.at[pl.ds(s0, ns), pl.ds(pl.multiple_of(off + r0, nr), nr)],
                    osem.at[j],
                ).start()

        def read_wait(j):
            pltpu.make_async_copy(xbuf.at[j], xbuf.at[j], rsem.at[j]).wait()

        def write_wait(j):
            pltpu.make_async_copy(obuf.at[j], obuf.at[j], osem.at[j]).wait()

        def compute(j):
            xv = xbuf[j].reshape(S * bu, C)
            r = jnp.dot(xv, wbuf[...], preferred_element_type=jnp.float32)
            obuf[j] = r.astype(obuf.dtype).reshape(S, bu, O)

        wcopy = pltpu.make_async_copy(w_hbm, wbuf, wsem.at[0])
        wcopy.start()
        read_start(0, 0)
        wcopy.wait()
        _loop(1, D, lambda j: read_start(0, j))

        def group(k):
            def read_phase(j):
                for t in range(2):
                    u = D + 2 * j + t
                    pl.when(u < P)(lambda u=u: read_start(k, u))
                read_wait(j)
                compute(j)

            _loop(0, half, read_phase)
            _loop(half, P - E, read_wait)
            _loop(0, D, lambda j: write_start(k, j))
            _loop(P - E, P, read_wait)

            def write_phase(j):
                compute(j)
                lo = jnp.minimum(D + 2 * (j - half), j)
                hi = jnp.minimum(D + 2 * (j - half) + 2, j + 1)
                for t in range(2):
                    pl.when(lo + t < hi)(lambda t=t: write_start(k, lo + t))

            _loop(half, P, write_phase)
            _loop(0, P - E, write_wait)
            pl.when(k + 1 < G)(lambda: _loop(0, D, lambda j: read_start(k + 1, j)))
            _loop(P - E, P, write_wait)

        _loop(0, G, group)

    out = pl.pallas_call(
        kernel,
        in_specs=[pl.BlockSpec(memory_space=pl.ANY), pl.BlockSpec(memory_space=pl.ANY)],
        out_specs=pl.BlockSpec(memory_space=pl.ANY),
        out_shape=jax.ShapeDtypeStruct((S, M // S, O), x.dtype),
        scratch_shapes=[
            pltpu.VMEM((P, S, bu, C), x.dtype),
            pltpu.VMEM((P, S, bu, O), x.dtype),
            pltpu.VMEM((C, O), w.dtype),
            pltpu.SemaphoreType.DMA((P,)),
            pltpu.SemaphoreType.DMA((P,)),
            pltpu.SemaphoreType.DMA((1,)),
        ],
        compiler_params=pltpu.CompilerParams(
            vmem_limit_bytes=120 * 1024 * 1024,
            disable_bounds_checks=True,
        ),
    )(x.reshape(S, M // S, C), w.reshape(C, O))
    return out.reshape(B, H, W, O)
```

```python
import jax
import jax.numpy as jnp
from jax import lax
import jax.experimental.pallas as pl
import jax.experimental.pallas.tpu as pltpu

_S = 8
_BU = 128
_PIECE = 32
_P = 72
_JS = 32
_DR = 3
_DW = 4
_E = 1


def _loop(lo, hi, fn):
    def body(j, carry):
        fn(j)
        return carry

    lax.fori_loop(lo, hi, body, None)


@jax.jit
def pallas_standalone__dilated_atrous__vision_kernel(x: jax.Array, w: jax.Array):
    B, H, W, C = x.shape
    O = w.shape[-1]
    M = B * H * W
    S, bu, P, JS, DR, DW, E = _S, _BU, _P, _JS, _DR, _DW, _E
    n = M // (S * bu)
    assert n * S * bu == M and n % P == 0
    G = n // P
    u0 = DR + 2 * JS
    assert u0 <= P - E and DW <= JS
    NS = DR + JS + 2

    def writes_issued(m, minimum):
        return minimum(DW + (13 * m) // 8, JS + m)

    def kernel(x_hbm, w_hbm, o_hbm, xbuf, obuf, wbuf, rsem, osem, wsem):
        def read_start(k, j):
            off = (k * P + j) * bu
            sem = rsem.at[jnp.where(j < JS, lax.rem(j, NS), jnp.where(j < P - E, NS, NS + 1))]
            for r0 in range(0, bu, _PIECE):
                rows = pl.ds(pl.multiple_of(off + r0, _PIECE), _PIECE)
                for s in range(S):
                    pltpu.make_async_copy(
                        x_hbm.at[s, rows], xbuf.at[j, s, pl.ds(r0, _PIECE)], sem
                    ).start(priority=1 - s % 2)

        def write_start(k, j):
            off = (k * P + j) * bu
            for r0 in range(0, bu, _PIECE):
                rows = pl.ds(pl.multiple_of(off + r0, _PIECE), _PIECE)
                pltpu.make_async_copy(
                    obuf.at[j, :, pl.ds(r0, _PIECE)], o_hbm.at[:, rows], osem.at[0]
                ).start()

        def wait_units(buf, count, sem):
            view = buf.at[pl.ds(0, count)]
            pltpu.make_async_copy(view, view, sem).wait()

        def compute(j):
            xv = xbuf[j].reshape(S * bu, C)
            r = jnp.dot(xv, wbuf[...], preferred_element_type=jnp.float32)
            obuf[j] = r.astype(obuf.dtype).reshape(S, bu, O)

        wcopy = pltpu.make_async_copy(w_hbm, wbuf, wsem.at[0])
        wcopy.start()
        _loop(0, DR, lambda j: read_start(0, j))
        wcopy.wait()

        def group(k):
            def read_step(j):
                _loop(DR + 2 * j, DR + 2 * j + 2, lambda u: read_start(k, u))
                wait_units(xbuf, 1, rsem.at[lax.rem(j, NS)])
                compute(j)

            _loop(0, JS, read_step)
            _loop(u0, P, lambda j: read_start(k, j))
            wait_units(xbuf, P - E - JS, rsem.at[NS])
            _loop(0, DW, lambda j: write_start(k, j))
            wait_units(xbuf, E, rsem.at[NS + 1])

            def write_step(m):
                compute(JS + m)
                _loop(
                    writes_issued(m, jnp.minimum),
                    writes_issued(m + 1, jnp.minimum),
                    lambda u: write_start(k, u),
                )

            _loop(0, P - JS, write_step)
            _loop(writes_issued(P - JS, min), P, lambda j: write_start(k, j))
            wait_units(obuf, P, osem.at[0])
            pl.when(k + 1 < G)(lambda: _loop(0, DR, lambda j: read_start(k + 1, j)))

        _loop(0, G, group)

    out = pl.pallas_call(
        kernel,
        in_specs=[pl.BlockSpec(memory_space=pl.ANY), pl.BlockSpec(memory_space=pl.ANY)],
        out_specs=pl.BlockSpec(memory_space=pl.ANY),
        out_shape=jax.ShapeDtypeStruct((S, M // S, O), x.dtype),
        scratch_shapes=[
            pltpu.VMEM((P, S, bu, C), x.dtype),
            pltpu.VMEM((P, S, bu, O), x.dtype),
            pltpu.VMEM((C, O), w.dtype),
            pltpu.SemaphoreType.DMA((NS + 2,)),
            pltpu.SemaphoreType.DMA((1,)),
            pltpu.SemaphoreType.DMA((1,)),
        ],
        compiler_params=pltpu.CompilerParams(
            vmem_limit_bytes=120 * 1024 * 1024,
            disable_bounds_checks=True,
        ),
    )(x.reshape(S, M // S, C), w.reshape(C, O))
    return out.reshape(B, H, W, O)
```

```python
import jax
import jax.numpy as jnp
from jax import lax
import jax.experimental.pallas as pl
import jax.experimental.pallas.tpu as pltpu

_S = 6
_BU = 192
_RD = 32
_WR = 48
_JS = 56
_DR = 3
_LW = 6
_DW = 4


def _loop(lo, hi, fn):
    def body(i, carry):
        fn(i)
        return carry

    lax.fori_loop(lo, hi, body, None)


@jax.jit
def pallas_standalone__dilated_atrous__vision_kernel(x: jax.Array, w: jax.Array):
    B, H, W, C = x.shape
    O = w.shape[-1]
    M = B * H * W
    S, bu, JS, DR, LW, DW = _S, _BU, _JS, _DR, _LW, _DW
    n = M // (S * bu)
    assert n * S * bu == M and DR + 2 * JS <= n and DW <= min(JS, LW)
    NX = max(n - JS, DR + JS + 1)
    NO = JS + 3

    def writes_issued(m, minimum):
        return minimum(DW + (13 * m) // 8, JS + m)

    assert all(JS + m - NO < max(writes_issued(m, min) - LW, 0) for m in range(n - JS))

    def kernel(x_hbm, w_hbm, o_hbm, xbuf, obuf, wbuf, rsem, osem):
        def read_start(u):
            slot, sem = lax.rem(u, NX), rsem.at[lax.rem(u, DR + 1)]
            for r0 in range(0, bu, _RD):
                rows = pl.ds(pl.multiple_of(u * bu + r0, 16), _RD)
                for s in range(S):
                    pltpu.make_async_copy(
                        x_hbm.at[s, rows], xbuf.at[slot, s, pl.ds(r0, _RD)], sem
                    ).start(priority=1 - s % 2)

        def write_start(u):
            slot, sem = lax.rem(u, NO), osem.at[lax.rem(u, LW + 1)]
            for r0 in range(0, bu, _WR):
                rows = pl.ds(pl.multiple_of(u * bu + r0, 16), _WR)
                pltpu.make_async_copy(
                    obuf.at[slot, :, pl.ds(r0, _WR)], o_hbm.at[:, rows], sem
                ).start()

        def read_wait(u):
            buf = xbuf.at[lax.rem(u, NX)]
            pltpu.make_async_copy(buf, buf, rsem.at[lax.rem(u, DR + 1)]).wait()

        def write_wait(u):
            buf = obuf.at[lax.rem(u, NO)]
            pltpu.make_async_copy(buf, buf, osem.at[lax.rem(u, LW + 1)]).wait()

        def read_advance(u):
            read_start(u)
            read_wait(u - DR)

        def write_advance(u):
            write_start(u)
            pl.when(u >= LW)(lambda: write_wait(u - LW))

        def compute(u):
            xv = xbuf[lax.rem(u, NX)].reshape(S * bu, C)
            r = jnp.dot(xv, wbuf[...], preferred_element_type=jnp.float32)
            obuf[lax.rem(u, NO)] = r.astype(obuf.dtype).reshape(S, bu, O)

        wcopy = pltpu.make_async_copy(w_hbm, wbuf, osem.at[0])
        wcopy.start()
        read_start(jnp.int32(0))
        wcopy.wait()
        _loop(1, DR, read_start)

        def read_step(j):
            _loop(DR + 2 * j, DR + 2 * j + 2, read_advance)
            compute(j)

        _loop(0, JS, read_step)
        _loop(DR + 2 * JS, n, read_advance)
        _loop(n - DR, n - 1, read_wait)
        _loop(0, DW, write_start)
        read_wait(jnp.int32(n - 1))

        def write_step(m):
            compute(JS + m)
            _loop(
                writes_issued(m, jnp.minimum),
                writes_issued(m + 1, jnp.minimum),
                write_advance,
            )

        _loop(0, n - JS, write_step)
        _loop(writes_issued(n - JS, min), n, write_advance)
        _loop(n - LW, n, write_wait)

    out = pl.pallas_call(
        kernel,
        in_specs=[pl.BlockSpec(memory_space=pl.ANY), pl.BlockSpec(memory_space=pl.ANY)],
        out_specs=pl.BlockSpec(memory_space=pl.ANY),
        out_shape=jax.ShapeDtypeStruct((S, M // S, O), x.dtype),
        scratch_shapes=[
            pltpu.VMEM((NX, S, bu, C), x.dtype),
            pltpu.VMEM((NO, S, bu, O), x.dtype),
            pltpu.VMEM((C, O), w.dtype),
            pltpu.SemaphoreType.DMA((DR + 1,)),
            pltpu.SemaphoreType.DMA((LW + 1,)),
        ],
        compiler_params=pltpu.CompilerParams(
            vmem_limit_bytes=120 * 1024 * 1024,
            disable_bounds_checks=True,
        ),
    )(x.reshape(S, M // S, C), w.reshape(C, O))
    return out.reshape(B, H, W, O)
```
